```python
import os as _os
_os.environ.setdefault("JAX_PLATFORMS", "cpu")
import jax
import jax.numpy as jnp

def _softmax(x, axis=-1):
    return jax.nn.softmax(x, axis=axis)
def _gelu(x):
    return jax.nn.gelu(x, approximate=True)
def _silu(x):
    return jax.nn.silu(x)
def _sigmoid(x):
    return jax.nn.sigmoid(x)
def _layernorm(x, axis=-1, eps=1e-5):
    m = jnp.mean(x, axis=axis, keepdims=True)
    v = jnp.var(x, axis=axis, keepdims=True)
    return (x - m) / jnp.sqrt(v + eps)
def _scatter_add(tgt, idx, src, axis=0):
    return tgt.at[idx].add(src)
def _segment_sum(src, seg, n):
    return jax.ops.segment_sum(src, seg, n)
class _Rng:
    def __init__(self, key):
        self._k = key
    def _next(self):
        self._k, sub = jax.random.split(self._k)
        return sub
    def normal(self, shape):
        return jax.random.normal(self._next(), shape, dtype=jnp.bfloat16)
    def randint(self, lo, hi, shape):
        return jax.random.randint(self._next(), shape, lo, hi, dtype=jnp.int32)
    def uniform(self, shape, lo=0.0, hi=1.0):
        return jax.random.uniform(self._next(), shape, jnp.bfloat16, lo, hi)
    def permutation(self, n):
        return jax.random.permutation(self._next(), n)


kernel_name = 'parallel_sum__sliding_local_dilated__geglu_ffn__prompt'

def setup_inputs():
    _rng = _Rng(jax.random.key(int.from_bytes(__import__("os").urandom(4), "little")))
    _w = (lambda a: (lambda t: t.astype(jnp.bfloat16) if jnp.issubdtype(t.dtype, jnp.floating) else t)(jnp.asarray(a)))
    def _A_setup():
        B, S, D = 1, 2048, 512
        return {
            "x": _w((lambda *s: _rng.normal(s) * 0.05)(B, S, D)),
            "wqkv": _w((lambda *s: _rng.normal(s) * 0.05)(D, 3 * D)),
            "wo": _w((lambda *s: _rng.normal(s) * 0.05)(D, D)),
        }
    _A_in = _A_setup()

    def _B_setup():
        B, S, D, F = 1, 2048, 512, 1376
        return {
            "x": _w((lambda *s: _rng.normal(s) * 0.05)(B, S, D)),
            "w_gate": _w((lambda *s: _rng.normal(s) * 0.05)(D, F)),
            "w_up": _w((lambda *s: _rng.normal(s) * 0.05)(D, F)),
            "w_down": _w((lambda *s: _rng.normal(s) * 0.05)(F, D)),
        }
    _B_in = _B_setup()

    return {
        "A_x": _A_in["x"],
        "A_wqkv": _A_in["wqkv"],
        "A_wo": _A_in["wo"],
        "B_x": _B_in["x"],
        "B_w_gate": _B_in["w_gate"],
        "B_w_up": _B_in["w_up"],
        "B_w_down": _B_in["w_down"],
    }

def reference(A_x, A_wqkv, A_wo, B_x, B_w_gate, B_w_up, B_w_down):
    def _A_ref(x, wqkv, wo):
        B, S, D = x.shape
        H = 32; Dh = D // H
        W, dil = 8, 2
        qkv = (lambda x, *d: x.transpose(*d))((x @ wqkv).reshape(B, S, 3, H, Dh), 2, 0, 3, 1, 4)
        q, k, v = qkv[0], qkv[1], qkv[2]
        scale = Dh ** -0.5
        pos = jnp.arange(S)
        off = jnp.arange(W) * dil
        idx = pos[:, None] - off[None, :]
        mask = idx >= 0
        idx_c = jnp.where(mask, idx, 0).reshape(-1)
        kg = k[:, :, idx_c, :].reshape(B, H, S, W, Dh)
        vg = v[:, :, idx_c, :].reshape(B, H, S, W, Dh)
        logits = jnp.einsum("bhsd,bhswd->bhsw", q, kg) * scale
        logits = jnp.where(mask[None, None, :, :], logits, -1e9)
        attn = _softmax(logits, axis=-1)
        o = jnp.einsum("bhsw,bhswd->bhsd", attn, vg)
        return (lambda x, *d: x.transpose(*d))(o, 0, 2, 1, 3).reshape(B, S, D) @ wo

    def _B_ref(x, w_gate, w_up, w_down):
        return (_gelu(x @ w_gate) * (x @ w_up)) @ w_down

    x = A_x
    xn = _layernorm(x, axis=-1)
    return x + _A_ref(xn, A_wqkv, A_wo) + _B_ref(xn, B_w_gate, B_w_up, B_w_down)
```

```python
import functools
import jax, jax.numpy as jnp
from jax import lax
import jax.experimental.pallas as pl
import jax.experimental.pallas.tpu as pltpu

S, D, F, H, DH, W, DIL = 2048, 512, 1376, 32, 16, 8, 2
HALO = 16
LOG2E = 1.4426950408889634
NT = (((1,), (1,)), ((), ()))
f32, bf16, u32 = jnp.float32, jnp.bfloat16, jnp.uint32
C0 = 0.7978845608028654
C1 = C0 * 0.044715


def make(TM=512, RC=16, FC=256, split=(1, 3, 5, 6), osplit=1):
    NB = S // TM
    ftiles = [(c, min(c + 128, F)) for c in range(0, F, 128)]

    def lane_block_transpose(tiles):
        lane = lax.broadcasted_iota(jnp.int32, tiles[0].shape, 1)
        b0 = (lane & 4) == 0
        b1 = (lane & 8) == 0
        a, b, c, d = tiles
        a1 = jnp.where(b0, a, pltpu.roll(b, 4, 1)); b1_ = jnp.where(b0, pltpu.roll(a, 128 - 4, 1), b)
        c1 = jnp.where(b0, c, pltpu.roll(d, 4, 1)); d1 = jnp.where(b0, pltpu.roll(c, 128 - 4, 1), d)
        a2 = jnp.where(b1, a1, pltpu.roll(c1, 8, 1)); c2 = jnp.where(b1, pltpu.roll(a1, 128 - 8, 1), c1)
        b2 = jnp.where(b1, b1_, pltpu.roll(d1, 8, 1)); d2 = jnp.where(b1, pltpu.roll(b1_, 128 - 8, 1), d1)
        return a2, b2, c2, d2

    def kernel(x_hbm, wqkv_hbm, wo_hbm, wg_hbm, wu_hbm, wd_hbm, o_hbm,
               x_s, xn_s, wqkv_r, wqkv_p, wo_r, wo_t, wo_p, wg, wu, wd, k_s, v_s, out_s, sems, osems):
        cnt = [0]
        def cp(src, dst):
            c = pltpu.make_async_copy(src, dst, sems.at[cnt[0]]); cnt[0] += 1
            return c
        x_cp = [cp(x_hbm.at[b * TM:(b + 1) * TM], x_s.at[b * TM:(b + 1) * TM]) for b in range(NB)]
        bounds = [0] + [min(s * 128, F) for s in split] + [F]
        gu_cp = [(cp(wg_hbm.at[a:b], wg.at[a:b]), cp(wu_hbm.at[a:b], wu.at[a:b])) for a, b in zip(bounds[:-1], bounds[1:])]
        qkv_cp = cp(wqkv_hbm, wqkv_r)
        wd_cp = cp(wd_hbm, wd)
        wo_cp = cp(wo_hbm, wo_r)
        order = [x_cp[0]] + [c for p in gu_cp[:3] for c in p] + [qkv_cp] + [c for p in gu_cp[3:] for c in p] + [x_cp[1], wd_cp, wo_cp] + x_cp[2:]
        for c in order:
            c.start()

        def prep_qkv(sec):
            for r in range(0, D, 64):
                tiles = [pltpu.bitcast(wqkv_r[r:r + 64, sec * D + j * 128: sec * D + (j + 1) * 128], u32) for j in range(4)]
                outs = lane_block_transpose(tiles)
                for j in range(4):
                    wqkv_p[r // 2:r // 2 + 32, sec * D + j * 128: sec * D + (j + 1) * 128] = outs[j]

        def prep_wo():
            wo_t[...] = pltpu.bitcast(wo_r[...], u32)
            for ii in range(4):
                for h8 in range(8):
                    parts = [wo_t[64 * j + 8 * h8 + 2 * ii: 64 * j + 8 * h8 + 2 * ii + 2, :] for j in range(4)]
                    wo_p[64 * ii + 8 * h8: 64 * ii + 8 * h8 + 8, :] = jnp.concatenate(parts, axis=0)

        def layernorm(row0):
            x = x_s[pl.ds(row0, TM), :].astype(f32)
            mu = jnp.mean(x, axis=-1, keepdims=True)
            xc = x - mu
            var = jnp.mean(xc * xc, axis=-1, keepdims=True)
            return (xc * lax.rsqrt(var + 1e-5)).astype(bf16)

        def ffn_tiles(xn, a, b):
            g = lax.dot_general(xn, wg[a:b, :], NT, preferred_element_type=f32)
            u = lax.dot_general(xn, wu[a:b, :], NT, preferred_element_type=f32)
            t = jnp.tanh(g * (C0 + C1 * (g * g)))
            hg = 0.5 * g
            return ((hg + hg * t) * u).astype(bf16)

        def ffn_range(xn, a, b):
            return [ffn_tiles(xn, c, min(c + FC, b)) for c in range(a, b, FC)]

        def qkv_sec(xn, sec):
            w = pltpu.bitcast(wqkv_p[:, sec * D:(sec + 1) * D], bf16)
            return jnp.dot(xn, w, preferred_element_type=f32)

        def store_kv(ref, val):
            for j in range(4):
                ref[j, HALO:HALO + TM, :] = val[:, 128 * j:128 * (j + 1)]

        def attention(q, first):
            lane = lax.broadcasted_iota(jnp.int32, (RC, 128), 1)
            e0 = (lane & 1) == 0
            e1 = (lane & 2) == 0
            q = q * (DH ** -0.5 * LOG2E)
            o_chunks = []
            for r in range(0, TM, RC):
                qj = [q[r:r + RC, 128 * j:128 * (j + 1)] for j in range(4)]
                ss = []
                for w in range(W):
                    st = HALO + r - DIL * w
                    t = qj[0] * k_s[0, st:st + RC, :]
                    for j in range(1, 4):
                        t = t + qj[j] * k_s[j, st:st + RC, :]
                    t = t + jnp.where(e0, pltpu.roll(t, 127, 1), pltpu.roll(t, 1, 1))
                    t = t + jnp.where(e1, pltpu.roll(t, 126, 1), pltpu.roll(t, 2, 1))
                    if first and r < DIL * (W - 1) and w > 0:
                        row = lax.broadcasted_iota(jnp.int32, (RC, 128), 0) + r
                        t = jnp.where(row >= DIL * w, t, -1e9)
                    ss.append(t)
                m = ss[0]
                for w in range(1, W):
                    m = jnp.maximum(m, ss[w])
                ps = [jnp.exp2(s - m) for s in ss]
                l = ps[0]
                for w in range(1, W):
                    l = l + ps[w]
                inv = 1.0 / l
                oj = []
                for j in range(4):
                    acc = None
                    for w in range(W):
                        st = HALO + r - DIL * w
                        term = ps[w] * v_s[j, st:st + RC, :]
                        acc = term if acc is None else acc + term
                    oj.append((acc * inv).astype(bf16))
                o_chunks.append(jnp.concatenate(oj, axis=1))
            o = jnp.concatenate(o_chunks, axis=0)
            k_s[:, 0:HALO, :] = k_s[:, TM:TM + HALO, :]
            v_s[:, 0:HALO, :] = v_s[:, TM:TM + HALO, :]
            return o

        def finish(b, row0, o, hs, next_row0):
            xn_s[...] = pltpu.bitcast(layernorm(next_row0), u32)
            h = jnp.concatenate(hs, axis=1)
            y = jnp.dot(h, wd[...], preferred_element_type=f32)
            y = y + jnp.dot(o, pltpu.bitcast(wo_p[...], bf16), preferred_element_type=f32)
            y = y + x_s[pl.ds(row0, TM), :].astype(f32)
            out_s[pl.ds(row0, TM), :] = y.astype(bf16)
            for p in range(osplit):
                cw = D // osplit
                pltpu.make_async_copy(out_s.at[pl.ds(row0, TM), p * cw:(p + 1) * cw], o_hbm.at[pl.ds(row0, TM), p * cw:(p + 1) * cw], osems.at[b * osplit + p]).start()

        k_s[:, 0:HALO, :] = jnp.zeros((4, HALO, 128), f32)
        v_s[:, 0:HALO, :] = jnp.zeros((4, HALO, 128), f32)
        x_cp[0].wait()
        xn = layernorm(0)
        hs = []
        for p in range(3):
            gu_cp[p][0].wait(); gu_cp[p][1].wait()
            hs += ffn_range(xn, bounds[p], bounds[p + 1])
        qkv_cp.wait(); gu_cp[3][0].wait(); gu_cp[3][1].wait()
        prep_qkv(0); prep_qkv(1); prep_qkv(2)
        hs += ffn_range(xn, bounds[3], bounds[4])
        q = qkv_sec(xn, 0)
        store_kv(k_s, qkv_sec(xn, 1))
        store_kv(v_s, qkv_sec(xn, 2))
        gu_cp[4][0].wait(); gu_cp[4][1].wait(); x_cp[1].wait(); wd_cp.wait(); wo_cp.wait()
        prep_wo()
        o = attention(q, True)
        hs += ffn_range(xn, bounds[4], bounds[5])
        finish(0, 0, o, hs, TM)
        for c in x_cp[2:]:
            c.wait()

        def body(b, carry):
            row0 = pl.multiple_of(b * TM, TM)
            nrow0 = pl.multiple_of(jnp.minimum(b + 1, NB - 1) * TM, TM)
            xn = pltpu.bitcast(xn_s[...], bf16)
            q = qkv_sec(xn, 0)
            store_kv(k_s, qkv_sec(xn, 1))
            store_kv(v_s, qkv_sec(xn, 2))
            o = attention(q, False)
            hs = ffn_range(xn, 0, F)
            finish(b, row0, o, hs, nrow0)
            return carry
        lax.fori_loop(1, NB, body, 0)
        for b in range(NB):
            for p in range(osplit):
                cw = D // osplit
                pltpu.make_async_copy(out_s.at[pl.ds(b * TM, TM), p * cw:(p + 1) * cw], o_hbm.at[pl.ds(b * TM, TM), p * cw:(p + 1) * cw], osems.at[b * osplit + p]).wait()

    def fn(A_x, A_wqkv, A_wo, B_x, B_w_gate, B_w_up, B_w_down):
        x = A_x.reshape(S, D)
        anyspec = pl.BlockSpec(memory_space=pl.ANY)
        out = pl.pallas_call(
            kernel,
            in_specs=[anyspec] * 6,
            out_specs=anyspec,
            out_shape=jax.ShapeDtypeStruct((S, D), bf16),
            scratch_shapes=[
                pltpu.VMEM((S, D), bf16), pltpu.VMEM((TM // 2, D), u32),
                pltpu.VMEM((D, 3 * D), bf16), pltpu.VMEM((D // 2, 3 * D), u32),
                pltpu.VMEM((D, D), bf16), pltpu.VMEM((D // 2, D), u32), pltpu.VMEM((D // 2, D), u32),
                pltpu.VMEM((F, D), bf16), pltpu.VMEM((F, D), bf16), pltpu.VMEM((F, D), bf16),
                pltpu.VMEM((4, HALO + TM, 128), f32), pltpu.VMEM((4, HALO + TM, 128), f32),
                pltpu.VMEM((S, D), bf16),
                pltpu.SemaphoreType.DMA((32,)), pltpu.SemaphoreType.DMA((NB * osplit,)),
            ],
            compiler_params=pltpu.CompilerParams(vmem_limit_bytes=100 * 1024 * 1024),
        )(x, A_wqkv, A_wo, B_w_gate.T, B_w_up.T, B_w_down)
        return out.reshape(1, S, D)
    return fn


_impl = make()


@jax.jit
def pallas_parallel_sum__sliding_local_dilated__geglu_ffn__prompt_kernel(
    A_x: jax.Array,
    A_wqkv: jax.Array,
    A_wo: jax.Array,
    B_x: jax.Array,
    B_w_gate: jax.Array,
    B_w_up: jax.Array,
    B_w_down: jax.Array,
):
    return _impl(A_x, A_wqkv, A_wo, B_x, B_w_gate, B_w_up, B_w_down)
```

```python
import contextlib
import jax, jax.numpy as jnp
from jax import lax
import jax.experimental.pallas as pl
import jax.experimental.pallas.tpu as pltpu

S, D, F, H, DH, W, DIL = 2048, 512, 1376, 32, 16, 8, 2
HALO = 16
FA = 1280
LOG2E = 1.4426950408889634
NT = (((1,), (1,)), ((), ()))
f32, bf16, u32 = jnp.float32, jnp.bfloat16, jnp.uint32
C0 = 0.7978845608028654
C1 = C0 * 0.044715


def make(T0=768, TM=640, RC=8, FC=512, lag=2, rpiece=128, early=112, scopes=False, pvg0=1, pvg=1, lag0=2, plan=1, lnt=896, lnt0=-1, glpos=1, FC0=128, accf=False, accf0=False, ucat=True):
    NL = (S - T0) // TM
    TX = max(T0, TM)

    def pieces_for(t):
        return [(0, t, 0, 256)] + [(r, rpiece, 256, 256) for r in range(0, t, rpiece)]
    NP = len(pieces_for(TX))

    def scope(name):
        return jax.named_scope(name) if scopes else contextlib.nullcontext()

    def block_transpose(tiles, axis, blk):
        n = tiles[0].shape[axis]
        idx = lax.broadcasted_iota(jnp.int32, tiles[0].shape, axis)
        m0 = (idx & blk) == 0
        m1 = (idx & (2 * blk)) == 0
        a, b, c, d = tiles

        def swap(p, q, m, s):
            return jnp.where(m, p, pltpu.roll(q, s, axis)), jnp.where(m, pltpu.roll(p, n - s, axis), q)
        a, b = swap(a, b, m0, blk)
        c, d = swap(c, d, m0, blk)
        a, c = swap(a, c, m1, 2 * blk)
        b, d = swap(b, d, m1, 2 * blk)
        return a, b, c, d

    def kernel(*refs):
        one = refs[-1]
        one[0] = 1

        def once(i, c):
            kernel_body(*refs[:-1])
            return c
        lax.fori_loop(0, one[0], once, 0)

    def kernel_body(x_hbm, wqkv_hbm, wo_hbm, wg_hbm, wu_hbm, wd_hbm, o_hbm,
                    x_s, xn_s, wqkv_r, wqkv_p, wo_r, wo_p, wg, wu, wd, k_s, v_s, z_s, *rest):
        outs, (sems, osems) = rest[:NP], rest[NP:]
        cnt = [0]

        def cp(src, dst):
            c = pltpu.make_async_copy(src, dst, sems.at[cnt[0]]); cnt[0] += 1
            return c
        xcp = lambda a, b: cp(x_hbm.at[a:b], x_s.at[a:b])
        gcp = lambda a, b: cp(wg_hbm.at[a:b], wg.at[a:b])
        ucp = lambda a, b: cp(wu_hbm.at[a:b], wu.at[a:b])
        if plan == 1:
            groups = [
                [xcp(0, 256)],
                [xcp(256, 384), gcp(FA, F), ucp(FA, F)],
                [xcp(384, 512), gcp(0, 128), ucp(0, 128)],
                [xcp(512, T0), gcp(128, 384), ucp(128, 256)],
                [ucp(256, 384), cp(wqkv_hbm, wqkv_r)],
                [gcp(384, FA), ucp(384, FA), cp(wd_hbm, wd.at[0:F]), cp(wo_hbm, wo_r), xcp(T0, T0 + TM)],
                [xcp(T0 + TM, S)],
            ]
        else:
            groups = [
                [xcp(0, 256)],
                [xcp(256, 384), gcp(FA, F), ucp(FA, F)],
                [xcp(384, 512), gcp(0, 128), ucp(0, 128)],
                [xcp(512, T0), gcp(128, 384), ucp(128, 384)],
                [cp(wqkv_hbm, wqkv_r), gcp(384, 512), ucp(384, 512)],
                [gcp(512, FA), ucp(512, FA), cp(wd_hbm, wd.at[0:F]), cp(wo_hbm, wo_r), xcp(T0, T0 + TM)],
                [xcp(T0 + TM, S)],
            ]
        for g in groups:
            for c in g:
                c.start()

        def wait(i):
            with scope(f"wait{i}"):
                for c in groups[i]:
                    c.wait()

        def fence(val, dep):
            zero = jnp.tile(z_s[...], (dep.shape[0] // 8, dep.shape[1] // 128))
            return pltpu.bitcast(pltpu.bitcast(val, u32) | (dep & zero), val.dtype)

        def prep_qkv(sec):
            for r in range(0, D, 64):
                tiles = [pltpu.bitcast(wqkv_r[r:r + 64, sec * D + j * 128: sec * D + (j + 1) * 128], u32) for j in range(4)]
                res = block_transpose(tiles, 1, 4)
                for j in range(4):
                    wqkv_p[r // 2:r // 2 + 32, sec * D + j * 128: sec * D + (j + 1) * 128] = res[j]

        def prep_wo():
            for h8 in range(8):
                tiles = [pltpu.bitcast(wo_r[128 * j + 16 * h8: 128 * j + 16 * h8 + 16, :], u32) for j in range(4)]
                res = block_transpose(tiles, 0, 2)
                for ii in range(4):
                    wo_p[64 * ii + 8 * h8: 64 * ii + 8 * h8 + 8, :] = res[ii]

        def layernorm(row0, n):
            x = x_s[pl.ds(row0, n), :].astype(f32)
            mu = jnp.mean(x, axis=-1, keepdims=True)
            xc = x - mu
            var = jnp.mean(xc * xc, axis=-1, keepdims=True)
            return (xc * lax.rsqrt(var + 1e-5)).astype(bf16)

        def gelu_mul(g, u):
            t = jnp.tanh(g * (C0 + C1 * (g * g)))
            hg = 0.5 * g
            return (hg + hg * t) * u

        def mmt(x, w, a, b):
            return lax.dot_general(x, w[a:b, :], NT, preferred_element_type=f32)

        def ffn_tiles(xn, a, b):
            return gelu_mul(mmt(xn, wg, a, b), mmt(xn, wu, a, b)).astype(bf16)

        def ffn_last_mm(xn):
            wl = jnp.concatenate([wg[FA:F, :], wu[FA:F, :]], axis=0)
            return lax.dot_general(wl, xn, NT, preferred_element_type=f32)

        def ffn_last_act(gut):
            fl = F - FA
            ht = gelu_mul(gut[:fl], gut[fl:])
            ht = jnp.concatenate([ht, jnp.zeros((128 - fl, ht.shape[1]), f32)], axis=0)
            return ht.T.astype(bf16)

        def ffn_range(xn, a, b, fc=FC):
            return [ffn_tiles(xn, c, min(c + fc, b)) for c in range(a, b, fc)]

        def qkv_sec(xn, sec):
            w = pltpu.bitcast(wqkv_p[:, sec * D:(sec + 1) * D], bf16)
            return jnp.dot(xn, w, preferred_element_type=f32)

        def store_kv(ref, val):
            for j in range(4):
                ref[j, HALO:HALO + val.shape[0], :] = val[:, 128 * j:128 * (j + 1)]

        class Attn:
            def __init__(self, q, first):
                self.q = q * (DH ** -0.5 * LOG2E)
                self.t = q.shape[0]
                self.first = first
                self.lag = lag0 if first else lag
                self.pvg = pvg0 if first else pvg
                self.toks = []
                self.ps = {}
                self.o = {}
                self.ptok = None

            def probs(self, r):
                lane = lax.broadcasted_iota(jnp.int32, (RC, 128), 1)
                e0 = (lane & 1) == 0
                e1 = (lane & 2) == 0
                qj = [self.q[r:r + RC, 128 * j:128 * (j + 1)] for j in range(4)]
                if len(self.toks) >= self.lag:
                    dep = self.toks[-self.lag] & jnp.tile(z_s[...], (RC // 8, 1))
                    qj = [pltpu.bitcast(pltpu.bitcast(a, u32) | dep, f32) for a in qj]
                ss = []
                for w in range(W):
                    st = HALO + r - DIL * w
                    t = qj[0] * k_s[0, st:st + RC, :]
                    for j in range(1, 4):
                        t = t + qj[j] * k_s[j, st:st + RC, :]
                    t = t + jnp.where(e0, pltpu.roll(t, 127, 1), pltpu.roll(t, 1, 1))
                    t = t + jnp.where(e1, pltpu.roll(t, 126, 1), pltpu.roll(t, 2, 1))
                    if self.first and r < DIL * (W - 1) and w > 0:
                        row = lax.broadcasted_iota(jnp.int32, (RC, 128), 0) + r
                        t = jnp.where(row >= DIL * w, t, -1e9 * LOG2E)
                    ss.append(t)
                m = ss[0]
                for w in range(1, W):
                    m = jnp.maximum(m, ss[w])
                ps = [jnp.exp2(s - m) for s in ss]
                l = ps[0]
                for w in range(1, W):
                    l = l + ps[w]
                inv = 1.0 / l
                self.ps[r] = (ps, inv)
                self.toks.append(pltpu.bitcast(inv, u32))

            def pv(self, r):
                ps, inv = self.ps.pop(r)
                oj = []
                for j in range(4):
                    acc = None
                    if (accf0 if self.first else accf):
                        pp = ps
                        if self.ptok is not None:
                            acc = pltpu.bitcast(self.ptok & jnp.tile(z_s[...], (RC // 8, 1)), f32)
                    elif j % self.pvg == 0:
                        pp = ps
                        if self.ptok is not None:
                            dep = self.ptok & jnp.tile(z_s[...], (RC // 8, 1))
                            pp = [pltpu.bitcast(pltpu.bitcast(a, u32) | dep, f32) for a in ps]
                    for w in range(W):
                        st = HALO + r - DIL * w
                        term = pp[w] * v_s[j, st:st + RC, :]
                        acc = term if acc is None else acc + term
                    on = acc * inv
                    oj.append(on)
                    self.ptok = pltpu.bitcast(on, u32)
                self.o[r] = jnp.concatenate(oj, axis=1)

            def run(self):
                t = self.t
                for r in range(0, t, RC):
                    if r not in self.ps:
                        self.probs(r)
                    self.pv(r)
                o = jnp.concatenate([self.o[r] for r in range(0, t, RC)], axis=0).astype(bf16)
                k_s[:, 0:HALO, :] = k_s[:, t:t + HALO, :]
                v_s[:, 0:HALO, :] = v_s[:, t:t + HALO, :]
                return o

        def out_copy(b, row0, t, p):
            r0, nr, c0, nc = pieces_for(t)[p]
            step = pieces_for(TX)[p][1]
            return pltpu.make_async_copy(outs[p].at[pl.ds(b * step, nr), :], o_hbm.at[pl.ds(row0 + r0, nr), c0:c0 + nc], osems.at[b * NP + p])

        def next_ln(val, next_row0):
            xnn = pltpu.bitcast(layernorm(next_row0, TM), u32)
            xn_s[...] = xnn
            if val.shape[0] > TM:
                return jnp.concatenate([fence(val[:TM], xnn), val[TM:]], axis=0)
            return fence(val, xnn)

        def finish(b, row0, o, hs):
            t = o.shape[0]
            h = jnp.concatenate(hs, axis=1)
            y = jnp.dot(o, pltpu.bitcast(wo_p[...], bf16), preferred_element_type=f32)
            y = y + jnp.dot(h, wd[...], preferred_element_type=f32)
            y = y + x_s[pl.ds(row0, t), :].astype(f32)
            y = y.astype(bf16)
            for p, (r0, nr, c0, nc) in enumerate(pieces_for(t)):
                step = pieces_for(TX)[p][1]
                st = b * step if isinstance(b, int) else pl.multiple_of(b * step, step)
                outs[p][pl.ds(st, nr), :] = y[r0:r0 + nr, c0:c0 + nc]
                out_copy(b, row0, t, p).start()

        def cat(xs):
            if ucat:
                return pltpu.bitcast(jnp.concatenate([pltpu.bitcast(a, u32) for a in xs], axis=0), bf16)
            return jnp.concatenate(xs, axis=0)
        pk = (lambda a: pltpu.bitcast(pltpu.bitcast(a, u32), bf16)) if ucat else (lambda a: a)

        def after(x, hl):
            n = hl.shape[0]
            top = jnp.concatenate([fence(x[:n, :128], pltpu.bitcast(hl, u32)), x[:n, 128:]], axis=1)
            return top if n == x.shape[0] else cat([top, x[n:]])

        k_s[:, 0:HALO, :] = jnp.zeros((4, HALO, 128), f32)
        v_s[:, 0:HALO, :] = jnp.zeros((4, HALO, 128), f32)
        z_s[...] = jnp.zeros((8, 128), u32)
        wd[F:FA + 128, :] = jnp.zeros((FA + 128 - F, D), bf16)
        wait(0)
        with scope("seg0"):
            n0 = pk(layernorm(0, 256))
        wait(1)
        with scope("seg1"):
            xa = cat([n0, layernorm(256, 128)])
            gla = ffn_last_mm(xa)
        wait(2)
        with scope("seg2"):
            hla = ffn_last_act(gla)
            nb_ = layernorm(384, 128)
            xab = cat([xa, nb_])
            g0 = mmt(xab, wg, 0, 128)
            glb = ffn_last_mm(nb_)
            u0 = mmt(after(xab, hla), wu, 0, 128)
            h0ab = pk(gelu_mul(g0, u0).astype(bf16))
        wait(3)
        with scope("seg3"):
            hlb = ffn_last_act(glb)
            nc_ = layernorm(512, T0 - 512)
            xn = cat([xab, nc_])
            h1 = ffn_tiles(xn, 128, 256)
            hlc = ffn_last_act(ffn_last_mm(nc_))
            h0c = pk(ffn_tiles(nc_, 0, 128))
            if plan == 1:
                g2 = mmt(after(xn, cat([hlb, hlc])), wg, 256, 384)
            else:
                g2 = mmt(xn, wg, 256, 384)
                h2 = gelu_mul(g2, mmt(after(xn, cat([hlb, hlc])), wu, 256, 384)).astype(bf16)
        wait(4)
        with scope("seg4"):
            prep_qkv(0); prep_qkv(1); prep_qkv(2)
            if plan == 1:
                hs = [h1, gelu_mul(g2, mmt(xn, wu, 256, 384)).astype(bf16)]
            else:
                hs = [h1, h2, ffn_tiles(xn, 384, 512)]
            q = qkv_sec(xn, 0)
            store_kv(k_s, qkv_sec(xn, 1))
            at = Attn(q, True)
            store_kv(v_s, qkv_sec(xn, 2))
            for r in range(0, early, RC):
                at.probs(r)
        wait(5)
        with scope("seg5"):
            prep_wo()
            hl = cat([hla, hlb, hlc])
            hs = [cat([h0ab, h0c])] + hs
            o = at.run()
            hs += ffn_range(xn, 384 if plan == 1 else 512, FA, FC0) + [hl]
            if lnt0 < 0:
                o = next_ln(o, T0)
            else:
                hh = jnp.concatenate(hs, axis=1)
                hs = ([hh[:, :lnt0]] if lnt0 else []) + [next_ln(hh[:, lnt0:lnt0 + D], T0)] + ([hh[:, lnt0 + D:]] if lnt0 + D < FA + 128 else [])
            finish(0, 0, o, hs)
        wait(6)

        def body(b, carry):
            row0 = pl.multiple_of(T0 + (b - 1) * TM, 128)
            nrow0 = pl.multiple_of(T0 + jnp.minimum(b, NL - 1) * TM, 128)
            xn = pltpu.bitcast(xn_s[...], bf16)
            if glpos == 3:
                store_kv(k_s, qkv_sec(xn, 1))
                hl = ffn_last_act(ffn_last_mm(xn))
                q = qkv_sec(xn, 0)
            else:
                q = qkv_sec(xn, 0)
                if glpos == 1: hl = ffn_last_act(ffn_last_mm(xn))
                store_kv(k_s, qkv_sec(xn, 1))
                if glpos == 2: hl = ffn_last_act(ffn_last_mm(xn))
            store_kv(v_s, qkv_sec(xn, 2))
            o = Attn(q, False).run()
            hs = ffn_range(xn, 0, FA) + [hl]
            if lnt < 0:
                o = next_ln(o, nrow0)
            else:
                hh = jnp.concatenate(hs, axis=1)
                hs = ([hh[:, :lnt]] if lnt else []) + [next_ln(hh[:, lnt:lnt + D], nrow0)] + ([hh[:, lnt + D:]] if lnt + D < FA + 128 else [])
            finish(b, row0, o, hs)
            return carry
        with scope("loop"):
            lax.fori_loop(1, NL + 1, body, 0)
        with scope("w_out"):
            for b in range(NL + 1):
                t = T0 if b == 0 else TM
                row0 = 0 if b == 0 else T0 + (b - 1) * TM
                for p in range(len(pieces_for(t))):
                    out_copy(b, row0, t, p).wait()

    def fn(A_x, A_wqkv, A_wo, B_x, B_w_gate, B_w_up, B_w_down):
        x = A_x.reshape(S, D)
        anyspec = pl.BlockSpec(memory_space=pl.ANY)
        out = pl.pallas_call(
            kernel,
            in_specs=[anyspec] * 6,
            out_specs=anyspec,
            out_shape=jax.ShapeDtypeStruct((S, D), bf16),
            scratch_shapes=[
                pltpu.VMEM((S, D), bf16), pltpu.VMEM((TM // 2, D), u32),
                pltpu.VMEM((D, 3 * D), bf16), pltpu.VMEM((D // 2, 3 * D), u32),
                pltpu.VMEM((D, D), bf16), pltpu.VMEM((D // 2, D), u32),
                pltpu.VMEM((F, D), bf16), pltpu.VMEM((F, D), bf16), pltpu.VMEM((FA + 128, D), bf16),
                pltpu.VMEM((4, HALO + TX, 128), f32), pltpu.VMEM((4, HALO + TX, 128), f32),
                pltpu.VMEM((8, 128), u32),
            ] + [pltpu.VMEM(((NL + 1) * nr, nc), bf16) for (_, nr, _, nc) in pieces_for(TX)] + [
                pltpu.SemaphoreType.DMA((19,)), pltpu.SemaphoreType.DMA(((NL + 1) * NP,)), pltpu.SMEM((1,), jnp.int32),
            ],
            compiler_params=pltpu.CompilerParams(vmem_limit_bytes=100 * 1024 * 1024, disable_bounds_checks=True, disable_semaphore_checks=True),
        )(x, A_wqkv, A_wo, B_w_gate.T, B_w_up.T, B_w_down)
        return out.reshape(1, S, D)
    return fn


_impl = make()


@jax.jit
def pallas_parallel_sum__sliding_local_dilated__geglu_ffn__prompt_kernel(
    A_x: jax.Array,
    A_wqkv: jax.Array,
    A_wo: jax.Array,
    B_x: jax.Array,
    B_w_gate: jax.Array,
    B_w_up: jax.Array,
    B_w_down: jax.Array,
):
    return _impl(A_x, A_wqkv, A_wo, B_x, B_w_gate, B_w_up, B_w_down)
```

```python
import jax
import jax.numpy as jnp
from jax import lax
import jax.experimental.pallas as pl
import jax.experimental.pallas.tpu as pltpu

S, D, F, DH, W, DIL = 2048, 512, 1376, 16, 8, 2
HALO = 16
FA = 1280
T0, TM = 768, 640
NL = (S - T0) // TM
RC = 8
LAG = 2
EARLY = 112
RP = 128
LOG2E = 1.4426950408889634
C0 = 0.7978845608028654
C1 = C0 * 0.044715
NT = (((1,), (1,)), ((), ()))
f32, bf16, u32 = jnp.float32, jnp.bfloat16, jnp.uint32


def _pieces(t):
    return [(0, t, 0, 256)] + [(r, RP, 256, 256) for r in range(0, t, RP)]


NP = len(_pieces(T0))


def _block_transpose(tiles, axis, blk):
    n = tiles[0].shape[axis]
    idx = lax.broadcasted_iota(jnp.int32, tiles[0].shape, axis)
    m0 = (idx & blk) == 0
    m1 = (idx & (2 * blk)) == 0
    a, b, c, d = tiles

    def swap(p, q, m, s):
        return (jnp.where(m, p, pltpu.roll(q, s, axis)),
                jnp.where(m, pltpu.roll(p, n - s, axis), q))

    a, b = swap(a, b, m0, blk)
    c, d = swap(c, d, m0, blk)
    a, c = swap(a, c, m1, 2 * blk)
    b, d = swap(b, d, m1, 2 * blk)
    return a, b, c, d


def _gelu_mul(g, u):
    t = jnp.tanh(g * (C0 + C1 * (g * g)))
    hg = 0.5 * g
    return (hg + hg * t) * u


def _pk(a):
    return pltpu.bitcast(pltpu.bitcast(a, u32), bf16)


def _cat(xs):
    return pltpu.bitcast(jnp.concatenate([pltpu.bitcast(a, u32) for a in xs], axis=0), bf16)


def _kernel(x_hbm, wqkv_hbm, wo_hbm, wg_hbm, wu_hbm, wd_hbm, o_hbm,
            x_s, xn_s, wqkv_r, wqkv_p, wo_r, wo_p, wg, wu, wd, k_s, v_s, z_s, *rest):
    outs, (sems, osems) = rest[:NP], rest[NP:]

    def out_copy(b, row0, t, p):
        r0, nr, c0, nc = _pieces(t)[p]
        step = _pieces(T0)[p][1]
        return pltpu.make_async_copy(outs[p].at[pl.ds(b * step, nr), :],
                                     o_hbm.at[pl.ds(row0 + r0, nr), c0:c0 + nc],
                                     osems.at[b * NP + p])

    def fence(val, dep):
        zero = jnp.tile(z_s[...], (dep.shape[0] // 8, dep.shape[1] // 128))
        return pltpu.bitcast(pltpu.bitcast(val, u32) | (dep & zero), val.dtype)

    def after(x, hl):
        n = hl.shape[0]
        top = jnp.concatenate([fence(x[:n, :128], pltpu.bitcast(hl, u32)), x[:n, 128:]], axis=1)
        return top if n == x.shape[0] else _cat([top, x[n:]])

    def prep_qkv(sec):
        for r in range(0, D, 64):
            cols = [slice(sec * D + j * 128, sec * D + (j + 1) * 128) for j in range(4)]
            res = _block_transpose([pltpu.bitcast(wqkv_r[r:r + 64, c], u32) for c in cols], 1, 4)
            for j in range(4):
                wqkv_p[r // 2:r // 2 + 32, cols[j]] = res[j]

    def prep_wo():
        for a in range(8):
            tiles = [pltpu.bitcast(wo_r[128 * j + 16 * a:128 * j + 16 * a + 16, :], u32) for j in range(4)]
            res = _block_transpose(tiles, 0, 2)
            for i in range(4):
                wo_p[64 * i + 8 * a:64 * i + 8 * a + 8, :] = res[i]

    def layernorm(row0, n):
        x = x_s[pl.ds(row0, n), :].astype(f32)
        mu = jnp.mean(x, axis=-1, keepdims=True)
        xc = x - mu
        var = jnp.mean(xc * xc, axis=-1, keepdims=True)
        return (xc * lax.rsqrt(var + 1e-5)).astype(bf16)

    def mmt(x, w, a, b):
        return lax.dot_general(x, w[a:b, :], NT, preferred_element_type=f32)

    def ffn_tiles(xn, a, b):
        return _gelu_mul(mmt(xn, wg, a, b), mmt(xn, wu, a, b)).astype(bf16)

    def ffn_range(xn, a, b, fc):
        return [ffn_tiles(xn, c, min(c + fc, b)) for c in range(a, b, fc)]

    def ffn_last_mm(xn):
        wl = jnp.concatenate([wg[FA:F, :], wu[FA:F, :]], axis=0)
        return lax.dot_general(wl, xn, NT, preferred_element_type=f32)

    def ffn_last_act(gut):
        fl = F - FA
        ht = _gelu_mul(gut[:fl], gut[fl:])
        ht = jnp.concatenate([ht, jnp.zeros((128 - fl, ht.shape[1]), f32)], axis=0)
        return ht.T.astype(bf16)

    def qkv_sec(xn, sec):
        w = pltpu.bitcast(wqkv_p[:, sec * D:(sec + 1) * D], bf16)
        return jnp.dot(xn, w, preferred_element_type=f32)

    def store_kv(ref, val):
        for j in range(4):
            ref[j, HALO:HALO + val.shape[0], :] = val[:, 128 * j:128 * (j + 1)]

    class Attn:
        def __init__(self, q, first):
            self.q = q * (DH ** -0.5 * LOG2E)
            self.first = first
            self.toks, self.ps, self.o, self.ptok = [], {}, {}, None

        @staticmethod
        def gate(vals, tok):
            dep = tok & z_s[...]
            return [pltpu.bitcast(pltpu.bitcast(a, u32) | dep, f32) for a in vals]

        def probs(self, r):
            lane = lax.broadcasted_iota(jnp.int32, (RC, 128), 1)
            e0 = (lane & 1) == 0
            e1 = (lane & 2) == 0
            qj = [self.q[r:r + RC, 128 * j:128 * (j + 1)] for j in range(4)]
            if len(self.toks) >= LAG:
                qj = self.gate(qj, self.toks[-LAG])
            ss = []
            for w in range(W):
                st = HALO + r - DIL * w
                t = qj[0] * k_s[0, st:st + RC, :]
                for j in range(1, 4):
                    t = t + qj[j] * k_s[j, st:st + RC, :]
                t = t + jnp.where(e0, pltpu.roll(t, 127, 1), pltpu.roll(t, 1, 1))
                t = t + jnp.where(e1, pltpu.roll(t, 126, 1), pltpu.roll(t, 2, 1))
                if self.first and r < DIL * (W - 1) and w > 0:
                    row = lax.broadcasted_iota(jnp.int32, (RC, 128), 0) + r
                    t = jnp.where(row >= DIL * w, t, -1e9 * LOG2E)
                ss.append(t)
            m = ss[0]
            for w in range(1, W):
                m = jnp.maximum(m, ss[w])
            ps = [jnp.exp2(s - m) for s in ss]
            l = ps[0]
            for w in range(1, W):
                l = l + ps[w]
            inv = 1.0 / l
            self.ps[r] = (ps, inv)
            self.toks.append(pltpu.bitcast(inv, u32))

        def pv(self, r):
            ps, inv = self.ps.pop(r)
            oj = []
            for j in range(4):
                pp = ps if self.ptok is None else self.gate(ps, self.ptok)
                acc = None
                for w in range(W):
                    st = HALO + r - DIL * w
                    term = pp[w] * v_s[j, st:st + RC, :]
                    acc = term if acc is None else acc + term
                on = acc * inv
                oj.append(on)
                self.ptok = pltpu.bitcast(on, u32)
            self.o[r] = jnp.concatenate(oj, axis=1)

        def run(self):
            t = self.q.shape[0]
            for r in range(0, t, RC):
                if r not in self.ps:
                    self.probs(r)
                self.pv(r)
            o = jnp.concatenate([self.o[r] for r in range(0, t, RC)], axis=0).astype(bf16)
            k_s[:, 0:HALO, :] = k_s[:, t:t + HALO, :]
            v_s[:, 0:HALO, :] = v_s[:, t:t + HALO, :]
            return o

    def next_ln(val, next_row0):
        xnn = pltpu.bitcast(layernorm(next_row0, TM), u32)
        xn_s[...] = xnn
        if val.shape[0] > TM:
            return jnp.concatenate([fence(val[:TM], xnn), val[TM:]], axis=0)
        return fence(val, xnn)

    def finish(b, row0, o, hs, y0=None):
        t = o.shape[0]
        h = jnp.concatenate(hs, axis=1)
        y = jnp.dot(o, pltpu.bitcast(wo_p[...], bf16), preferred_element_type=f32)
        if y0 is None:
            y = y + jnp.dot(h, wd[...], preferred_element_type=f32)
        else:
            y = y + (jnp.dot(h, wd[384:FA, :], preferred_element_type=f32) + y0)
        y = y + x_s[pl.ds(row0, t), :].astype(f32)
        y = y.astype(bf16)
        for p, (r0, nr, c0, nc) in enumerate(_pieces(t)):
            step = _pieces(T0)[p][1]
            st = b * step if isinstance(b, int) else pl.multiple_of(b * step, step)
            outs[p][pl.ds(st, nr), :] = y[r0:r0 + nr, c0:c0 + nc]
            out_copy(b, row0, t, p).start()

    @pl.when(pl.program_id(0) == 0)
    def _compute():
        cnt = [0]

        def cp(src, dst):
            c = pltpu.make_async_copy(src, dst, sems.at[cnt[0]])
            cnt[0] += 1
            return c

        xcp = lambda a, b: cp(x_hbm.at[a:b], x_s.at[a:b])
        gcp = lambda a, b: cp(wg_hbm.at[a:b], wg.at[a:b])
        ucp = lambda a, b: cp(wu_hbm.at[a:b], wu.at[a:b])
        groups = [
            [xcp(0, 256)],
            [xcp(256, 384), gcp(FA, F), ucp(FA, F)],
            [xcp(384, 512), gcp(0, 128), ucp(0, 128)],
            [xcp(512, T0), gcp(128, 384), ucp(128, 256)],
            [ucp(256, 384), cp(wqkv_hbm, wqkv_r)],
            [gcp(384, FA), ucp(384, FA), cp(wd_hbm, wd.at[0:F]), cp(wo_hbm, wo_r), xcp(T0, T0 + TM)],
            [xcp(T0 + TM, S)],
        ]
        for g in groups:
            for c in g:
                c.start()

        def wait(i):
            for c in groups[i]:
                c.wait()

        k_s[:, 0:HALO, :] = jnp.zeros((4, HALO, 128), f32)
        v_s[:, 0:HALO, :] = jnp.zeros((4, HALO, 128), f32)
        z_s[...] = jnp.zeros((8, 128), u32)
        wd[F:FA + 128, :] = jnp.zeros((FA + 128 - F, D), bf16)
        wait(0)
        n0 = _pk(layernorm(0, 256))
        wait(1)
        xa = _cat([n0, layernorm(256, 128)])
        gla = ffn_last_mm(xa)
        wait(2)
        hla = ffn_last_act(gla)
        nb = layernorm(384, 128)
        xab = _cat([xa, nb])
        g0 = mmt(xab, wg, 0, 128)
        glb = ffn_last_mm(nb)
        u0 = mmt(after(xab, hla), wu, 0, 128)
        h0ab = _pk(_gelu_mul(g0, u0).astype(bf16))
        wait(3)
        hlb = ffn_last_act(glb)
        nc = layernorm(512, T0 - 512)
        xn = _cat([xab, nc])
        h1 = ffn_tiles(xn, 128, 256)
        hlc = ffn_last_act(ffn_last_mm(nc))
        h0c = _pk(ffn_tiles(nc, 0, 128))
        g2 = mmt(after(xn, _cat([hlb, hlc])), wg, 256, 384)
        wait(4)
        for sec in range(3):
            prep_qkv(sec)
        hs = [h1, _gelu_mul(g2, mmt(xn, wu, 256, 384)).astype(bf16)]
        q = qkv_sec(xn, 0)
        store_kv(k_s, qkv_sec(xn, 1))
        at = Attn(q, True)
        store_kv(v_s, qkv_sec(xn, 2))
        for r in range(0, EARLY, RC):
            at.probs(r)
        wait(5)
        prep_wo()
        hl = _cat([hla, hlb, hlc])
        hs = [_cat([h0ab, h0c])] + hs
        y0 = jnp.dot(jnp.concatenate(hs + [hl], axis=1),
                     jnp.concatenate([wd[0:384, :], wd[FA:FA + 128, :]], axis=0),
                     preferred_element_type=f32)
        o = at.run()
        hs = ffn_range(xn, 384, FA, 256)
        o = next_ln(o, T0)
        finish(0, 0, o, hs, y0)
        wait(6)

        def body(b, carry):
            row0 = pl.multiple_of(T0 + (b - 1) * TM, 128)
            nrow0 = pl.multiple_of(T0 + jnp.minimum(b, NL - 1) * TM, 128)
            xn = pltpu.bitcast(xn_s[...], bf16)
            q = qkv_sec(xn, 0)
            hl = ffn_last_act(ffn_last_mm(xn))
            store_kv(k_s, qkv_sec(xn, 1))
            store_kv(v_s, qkv_sec(xn, 2))
            o = Attn(q, False).run()
            hh = jnp.concatenate(ffn_range(xn, 0, FA, 512) + [hl], axis=1)
            c = FA + 128 - D
            finish(b, row0, o, [hh[:, :c], next_ln(hh[:, c:], nrow0)])
            return carry

        lax.fori_loop(1, NL + 1, body, 0)

    @pl.when(pl.program_id(0) == 1)
    def _drain():
        for b in range(NL + 1):
            t = T0 if b == 0 else TM
            row0 = 0 if b == 0 else T0 + (b - 1) * TM
            for p in range(len(_pieces(t))):
                out_copy(b, row0, t, p).wait()


def _call(A_x, A_wqkv, A_wo, B_x, B_w_gate, B_w_up, B_w_down):
    del B_x
    hbm = pl.BlockSpec(memory_space=pl.ANY)
    out = pl.pallas_call(
        _kernel,
        grid=(2,),
        in_specs=[hbm] * 6,
        out_specs=hbm,
        out_shape=jax.ShapeDtypeStruct((S, D), bf16),
        scratch_shapes=[
            pltpu.VMEM((S, D), bf16), pltpu.VMEM((TM // 2, D), u32),
            pltpu.VMEM((D, 3 * D), bf16), pltpu.VMEM((D // 2, 3 * D), u32),
            pltpu.VMEM((D, D), bf16), pltpu.VMEM((D // 2, D), u32),
            pltpu.VMEM((F, D), bf16), pltpu.VMEM((F, D), bf16), pltpu.VMEM((FA + 128, D), bf16),
            pltpu.VMEM((4, HALO + T0, 128), f32), pltpu.VMEM((4, HALO + T0, 128), f32),
            pltpu.VMEM((8, 128), u32),
        ] + [pltpu.VMEM(((NL + 1) * nr, nc), bf16) for (_, nr, _, nc) in _pieces(T0)] + [
            pltpu.SemaphoreType.DMA((18,)), pltpu.SemaphoreType.DMA(((NL + 1) * NP,)),
        ],
        compiler_params=pltpu.CompilerParams(
            dimension_semantics=("arbitrary",), vmem_limit_bytes=100 * 1024 * 1024,
            disable_bounds_checks=True, disable_semaphore_checks=True),
    )(A_x.reshape(S, D), A_wqkv, A_wo, B_w_gate.T, B_w_up.T, B_w_down)
    return out.reshape(1, S, D)


@jax.jit
def pallas_parallel_sum__sliding_local_dilated__geglu_ffn__prompt_kernel(
    A_x: jax.Array,
    A_wqkv: jax.Array,
    A_wo: jax.Array,
    B_x: jax.Array,
    B_w_gate: jax.Array,
    B_w_up: jax.Array,
    B_w_down: jax.Array,
):
    return _call(A_x, A_wqkv, A_wo, B_x, B_w_gate, B_w_up, B_w_down)
```
